```python
import os as _os
_os.environ.setdefault("JAX_PLATFORMS", "cpu")
import jax
import jax.numpy as jnp

def _softmax(x, axis=-1):
    return jax.nn.softmax(x, axis=axis)
def _gelu(x):
    return jax.nn.gelu(x, approximate=True)
def _silu(x):
    return jax.nn.silu(x)
def _sigmoid(x):
    return jax.nn.sigmoid(x)
def _layernorm(x, axis=-1, eps=1e-5):
    m = jnp.mean(x, axis=axis, keepdims=True)
    v = jnp.var(x, axis=axis, keepdims=True)
    return (x - m) / jnp.sqrt(v + eps)
def _scatter_add(tgt, idx, src, axis=0):
    return tgt.at[idx].add(src)
def _segment_sum(src, seg, n):
    return jax.ops.segment_sum(src, seg, n)
class _Rng:
    def __init__(self, key):
        self._k = key
    def _next(self):
        self._k, sub = jax.random.split(self._k)
        return sub
    def normal(self, shape):
        return jax.random.normal(self._next(), shape, dtype=jnp.bfloat16)
    def randint(self, lo, hi, shape):
        return jax.random.randint(self._next(), shape, lo, hi, dtype=jnp.int32)
    def uniform(self, shape, lo=0.0, hi=1.0):
        return jax.random.uniform(self._next(), shape, jnp.bfloat16, lo, hi)
    def permutation(self, n):
        return jax.random.permutation(self._next(), n)


kernel_name = 'standalone__mha_softmax__decode'

def setup_inputs():
    _rng = _Rng(jax.random.key(int.from_bytes(__import__("os").urandom(4), "little")))
    _w = (lambda a: (lambda t: t.astype(jnp.bfloat16) if jnp.issubdtype(t.dtype, jnp.floating) else t)(jnp.asarray(a)))
    B, H, Sq, Sk, D = 1, 32, 1, 8192, 128
    return {
        "q": _w((lambda *s: _rng.normal(s) * 0.8)(B, H, Sq, D)),
        "k": _w((lambda *s: _rng.normal(s) * 0.8)(B, H, Sk, D)),
        "v": _w((lambda *s: _rng.normal(s) * 0.05)(B, H, Sk, D)),
    }

def reference(q, k, v):
    scale = q.shape[-1] ** -0.5
    scores = jnp.einsum("bhqd,bhkd->bhqk", q, k) * scale
    p = _softmax(scores, axis=-1)
    return jnp.einsum("bhqk,bhkd->bhqd", p, v)
```

```python
import math

import jax
import jax.numpy as jnp
from jax import lax
import jax.experimental.pallas as pl
import jax.experimental.pallas.tpu as pltpu

_TILE = 128
_GROUP = 8
_DMA_HEADS = 2
_DMA_ROWS = 64
_LOOKAHEAD = 3
_NBUF = 4


def _attention_kernel(q_hbm, k_hbm, v_hbm, o_hbm, buf, q_buf, s_buf, o_buf, sems, tail_sems, io_sem):
    num_heads, seq, dim = k_hbm.shape
    num_chunks = seq // _TILE
    num_groups = num_heads // _GROUP
    exp2_scale = dim**-0.5 * math.log2(math.e)
    pieces = [(h, j) for j in range(0, _TILE, _DMA_ROWS) for h in range(0, num_heads, _DMA_HEADS)]

    def start_piece(src, t, slot, h, j, sem, priority):
        row0 = t * _TILE + j
        if not isinstance(row0, int):
            row0 = pl.multiple_of(row0, _DMA_ROWS)
        pltpu.make_async_copy(
            src.at[pl.ds(h, _DMA_HEADS), pl.ds(row0, _DMA_ROWS)],
            buf.at[slot, pl.ds(h, _DMA_HEADS), pl.ds(j, _DMA_ROWS)],
            sem,
        ).start(priority=priority)

    def start_chunk(src, t, slot):
        for n, (h, j) in enumerate(pieces):
            start_piece(src, t, slot, h, j, sems.at[slot], n % 2)

    def start_last_chunk(slot):
        for n, (h, j) in enumerate(sorted(pieces, key=lambda p: p[0] // _GROUP)):
            start_piece(v_hbm, num_chunks - 1, slot, h, j, tail_sems.at[h // _GROUP], n % 2)

    def wait_chunk(slot):
        pltpu.make_async_copy(buf.at[slot], buf.at[slot], sems.at[slot]).wait()

    start_chunk(k_hbm, 0, 0)
    q_copy = pltpu.make_async_copy(q_hbm, q_buf, io_sem)
    q_copy.start()
    for t in range(1, _LOOKAHEAD):
        start_chunk(k_hbm, t, t)
    q_copy.wait()

    sublane = lax.broadcasted_iota(jnp.int32, (_GROUP, _TILE), 0)
    q_f32 = q_buf[...].astype(jnp.float32)
    q_groups = [q_f32[g * _GROUP:(g + 1) * _GROUP].astype(q_buf.dtype) for g in range(num_groups)]

    def per_head_matmul(lhs, slot, g, dims):
        out = None
        for i in range(_GROUP):
            r = lax.dot_general(lhs, buf[slot, g * _GROUP + i], dims, preferred_element_type=jnp.float32)
            out = r if out is None else jnp.where(sublane == i, r, out)
        return out

    qk_dims = (((1,), (1,)), ((), ()))
    pv_dims = (((1,), (0,)), ((), ()))

    def k_step(next_src, next_offset):
        def body(t, lane_max):
            slot = t & (_NBUF - 1)
            wait_chunk(slot)
            start_chunk(next_src, t + next_offset, (t + _LOOKAHEAD) & (_NBUF - 1))
            new_max = []
            for g in range(num_groups):
                s = per_head_matmul(q_groups[g], slot, g, qk_dims)
                s_buf[t, pl.ds(g * _GROUP, _GROUP), :] = s
                new_max.append(jnp.maximum(lane_max[g], s))
            return new_max
        return body

    lane_max = [jnp.full((_GROUP, _TILE), -jnp.inf, jnp.float32)] * num_groups
    lane_max = lax.fori_loop(0, num_chunks - _LOOKAHEAD, k_step(k_hbm, _LOOKAHEAD), lane_max)
    lane_max = lax.fori_loop(
        num_chunks - _LOOKAHEAD, num_chunks, k_step(v_hbm, _LOOKAHEAD - num_chunks), lane_max)
    row_max = [
        jnp.broadcast_to(jnp.max(m, axis=1, keepdims=True), (_GROUP, _TILE)) for m in lane_max]

    def probs(t):
        return [
            jnp.exp2((s_buf[t, pl.ds(g * _GROUP, _GROUP), :] - row_max[g]) * exp2_scale)
            for g in range(num_groups)]

    def v_step(start_next):
        def body(t, carry):
            acc, lane_sum = carry
            slot = t & (_NBUF - 1)
            p = probs(t)
            wait_chunk(slot)
            start_next(t + _LOOKAHEAD, (t + _LOOKAHEAD) & (_NBUF - 1))
            acc = [
                acc[g] + per_head_matmul(p[g].astype(buf.dtype), slot, g, pv_dims)
                for g in range(num_groups)]
            return acc, [a + b for a, b in zip(lane_sum, p)]
        return body

    zeros = [jnp.zeros((_GROUP, _TILE), jnp.float32)] * num_groups
    last = num_chunks - 1
    carry = lax.fori_loop(
        0, last - _LOOKAHEAD, v_step(lambda t, slot: start_chunk(v_hbm, t, slot)), (zeros, zeros))
    carry = v_step(lambda t, slot: start_last_chunk(slot))(last - _LOOKAHEAD, carry)
    acc, lane_sum = lax.fori_loop(last - _LOOKAHEAD + 1, last, v_step(lambda t, slot: None), carry)

    slot = last & (_NBUF - 1)
    p = probs(last)
    inv_sum = [1.0 / jnp.sum(a + b, axis=1, keepdims=True) for a, b in zip(lane_sum, p)]
    out = []
    for g in range(num_groups):
        tiles = buf.at[slot, pl.ds(g * _GROUP, _GROUP)]
        pltpu.make_async_copy(tiles, tiles, tail_sems.at[g]).wait()
        out.append((acc[g] + per_head_matmul(p[g].astype(buf.dtype), slot, g, pv_dims)) * inv_sum[g])
    o_buf[...] = jnp.concatenate(out, axis=0).astype(o_buf.dtype)
    o_copy = pltpu.make_async_copy(o_buf, o_hbm, io_sem)
    o_copy.start()
    o_copy.wait()


@jax.jit
def pallas_standalone__mha_softmax__decode_kernel(q: jax.Array, k: jax.Array, v: jax.Array):
    batch, heads, q_len, dim = q.shape
    seq = k.shape[2]
    num_heads = batch * heads
    assert q_len == 1 and dim == _TILE and seq % _TILE == 0 and num_heads % _GROUP == 0
    out = pl.pallas_call(
        _attention_kernel,
        in_specs=[pl.BlockSpec(memory_space=pl.ANY)] * 3,
        out_specs=pl.BlockSpec(memory_space=pl.ANY),
        out_shape=jax.ShapeDtypeStruct((num_heads, dim), q.dtype),
        scratch_shapes=[
            pltpu.VMEM((_NBUF, num_heads, _TILE, dim), k.dtype),
            pltpu.VMEM((num_heads, dim), q.dtype),
            pltpu.VMEM((seq // _TILE, num_heads, _TILE), jnp.float32),
            pltpu.VMEM((num_heads, dim), q.dtype),
            pltpu.SemaphoreType.DMA((_NBUF,)),
            pltpu.SemaphoreType.DMA((num_heads // _GROUP,)),
            pltpu.SemaphoreType.DMA(()),
        ],
        compiler_params=pltpu.CompilerParams(
            disable_bounds_checks=True, disable_semaphore_checks=True),
    )(q.reshape(num_heads, dim), k.reshape(num_heads, seq, dim), v.reshape(num_heads, seq, dim))
    return out.reshape(q.shape)
```

```python
import math

import jax
import jax.numpy as jnp
from jax import lax
import jax.experimental.pallas as pl
import jax.experimental.pallas.tpu as pltpu

_TILE = 128
_UNIT = 64
_PIECE = 32
_SUBLANES = 8
_HEADS = 16
_STRIDE = 4
_LOW_SEGS = 3
_AHEAD_LOW = 6
_AHEAD_HIGH = 3
_NBUF = 8

_QK_DIMS = (((1,), (1,)), ((), ()))
_PV_DIMS = (((1,), (0,)), ((), ()))


def _attention_kernel(
    q_hbm, k_hbm, v_hbm, o_hbm,
    buf, early_buf, late_buf, q_buf, s_buf, p_buf, o_buf,
    sems, early_sem, late_sems, io_sem,
):
    seq = k_hbm.shape[1] // _STRIDE
    num_chunks = seq // _TILE
    last = num_chunks - 1
    segs = _HEADS // _STRIDE
    groups = _HEADS // _SUBLANES
    num_passes = q_hbm.shape[0] // _HEADS
    exp2_scale = q_hbm.shape[1] ** -0.5 * math.log2(math.e)
    streams = [(src, x) for x in range(num_passes) for src in (k_hbm, v_hbm)]

    def source(stream, t, half, b, seg, num_segs, offset=0, rows=_UNIT):
        src, x = stream
        unit = (2 * t) ^ (half * (num_chunks + 1))
        row0 = b * seq + unit * _UNIT + offset
        if not isinstance(row0, int):
            row0 = pl.multiple_of(row0, rows)
        return src.at[pl.ds(x * segs + seg, num_segs), pl.ds(row0, rows)]

    def chunk_dma(stream, t, seg, num_segs, priority):
        def start(half, b):
            slot = t & (_NBUF - 1)
            pltpu.make_async_copy(
                source(stream, t, half, b, seg, num_segs),
                buf.at[slot, pl.ds(seg, num_segs), b, pl.ds(half * _UNIT, _UNIT)],
                sems.at[slot],
            ).start(priority=priority)
        return start

    def low(stream, t):
        return chunk_dma(stream, t, 0, _LOW_SEGS, 1)

    def high(stream, t):
        return chunk_dma(stream, t, _LOW_SEGS, segs - _LOW_SEGS, 0)

    def issue(*starts):
        for half in range(2):
            for b in range(_STRIDE):
                for start in starts:
                    start(half, b)

    def wait(ref, sem):
        pltpu.make_async_copy(ref, ref, sem).wait()

    q_copy = pltpu.make_async_copy(q_hbm, q_buf, io_sem)
    for t in range(_AHEAD_LOW):
        t_high = t - (_AHEAD_LOW - _AHEAD_HIGH)
        if t_high < 0:
            issue(low(streams[0], t))
        else:
            issue(low(streams[0], t), high(streams[0], t_high))
        if t_high == 0:
            q_copy.start()
    q_copy.wait()

    sublane = lax.broadcasted_iota(jnp.int32, (_SUBLANES, _TILE), 0)
    q_f32 = q_buf[...].astype(jnp.float32)

    def per_head_matmul(lhs, t, dims):
        results = []
        for g in range(groups):
            out = None
            for i in range(_SUBLANES):
                h = g * _SUBLANES + i
                tile = buf[t & (_NBUF - 1), h // _STRIDE, h % _STRIDE]
                r = lax.dot_general(lhs[g], tile, dims, preferred_element_type=jnp.float32)
                out = r if out is None else jnp.where(sublane == i, r, out)
            results.append(out)
        return results

    def advance(t, starts):
        slot = t & (_NBUF - 1)
        wait(buf.at[slot], sems.at[slot])
        issue(*starts)

    def run_stream(step, carry, this, following):
        def steady(t, c):
            return step(t, c, (low(this, t + _AHEAD_LOW), high(this, t + _AHEAD_HIGH)))

        def low_moved_on(t, c):
            return step(t, c, (low(following, t + _AHEAD_LOW - num_chunks), high(this, t + _AHEAD_HIGH)))

        def both_moved_on(t, c):
            return step(t, c, (low(following, t + _AHEAD_LOW - num_chunks),
                               high(following, t + _AHEAD_HIGH - num_chunks)))

        carry = lax.fori_loop(0, num_chunks - _AHEAD_LOW, steady, carry)
        carry = lax.fori_loop(num_chunks - _AHEAD_LOW, num_chunks - _AHEAD_HIGH, low_moved_on, carry)
        return lax.fori_loop(num_chunks - _AHEAD_HIGH, num_chunks, both_moved_on, carry)

    for x in range(num_passes):
        keys, values = streams[2 * x], streams[2 * x + 1]
        q = [
            q_f32[x * _HEADS + g * _SUBLANES:x * _HEADS + (g + 1) * _SUBLANES].astype(q_buf.dtype)
            for g in range(groups)]

        def score_step(t, lane_max, starts):
            advance(t, starts)
            s = per_head_matmul(q, t, _QK_DIMS)
            for g in range(groups):
                s_buf[t, g] = s[g]
            return [jnp.maximum(m, sg) for m, sg in zip(lane_max, s)]

        lane_max = run_stream(
            score_step, [jnp.full((_SUBLANES, _TILE), -jnp.inf, jnp.float32)] * groups, keys, values)
        row_max = [
            jnp.broadcast_to(jnp.max(m, axis=1, keepdims=True), (_SUBLANES, _TILE)) for m in lane_max]

        def probs(t):
            return [jnp.exp2((s_buf[t, g] - row_max[g]) * exp2_scale) for g in range(groups)]

        def add(xs, ys):
            return [a + b for a, b in zip(xs, ys)]

        def value_step(t, carry, starts):
            acc, lane_sum = carry
            p = probs(t)
            advance(t, starts)
            pv = per_head_matmul([pg.astype(buf.dtype) for pg in p], t, _PV_DIMS)
            return add(acc, pv), add(lane_sum, p)

        zeros = [jnp.zeros((_SUBLANES, _TILE), jnp.float32)] * groups
        if x + 1 < num_passes:
            acc, lane_sum = run_stream(value_step, (zeros, zeros), values, streams[2 * x + 2])
            out = [a / jnp.sum(s, axis=1, keepdims=True) for a, s in zip(acc, lane_sum)]
            o_buf[pl.ds(x * _HEADS, _HEADS)] = jnp.concatenate(out, axis=0).astype(o_buf.dtype)
            continue

        def last_low(half, b):
            if half == 0:
                pltpu.make_async_copy(
                    source(values, last, half, b, 0, _LOW_SEGS),
                    early_buf.at[b, pl.ds(0, _LOW_SEGS)], early_sem).start(priority=1)
            else:
                late_piece(half, b)

        def last_high(half, b):
            n = segs - _LOW_SEGS
            pltpu.make_async_copy(
                source(values, last, half, b, _LOW_SEGS, n),
                early_buf.at[b, pl.ds(_LOW_SEGS + half * n, n)], early_sem).start(priority=0)

        pieces = [
            (b, seg, offset)
            for b in range(_STRIDE) for seg in range(_LOW_SEGS) for offset in range(0, _UNIT, _PIECE)]
        num_slots = _STRIDE * (1 + 2 * (_AHEAD_LOW - _AHEAD_HIGH))
        slots = [
            pieces[len(pieces) * i // num_slots:len(pieces) * (i + 1) // num_slots]
            for i in range(num_slots)]

        def late_piece(half, b):
            for pb, seg, offset in slots.pop(0):
                pltpu.make_async_copy(
                    source(values, last, 1, pb, seg, 1, offset, _PIECE),
                    late_buf.at[pb, pl.ds(seg, 1), pl.ds(offset, _PIECE)], late_sems.at[pb]).start(priority=1)

        carry = lax.fori_loop(
            0, last - _AHEAD_LOW,
            lambda t, c: value_step(t, c, (low(values, t + _AHEAD_LOW), high(values, t + _AHEAD_HIGH))),
            (zeros, zeros))
        for t in range(last - _AHEAD_LOW, num_chunks - _AHEAD_HIGH):
            carry = value_step(t, carry, (
                last_low if t + _AHEAD_LOW == last else late_piece,
                last_high if t + _AHEAD_HIGH == last else high(values, t + _AHEAD_HIGH)))
        assert not slots

        acc, lane_sum = carry
        for t in range(num_chunks - _AHEAD_HIGH, num_chunks):
            lane_sum = add(lane_sum, probs(t))
        inv_sum = [1.0 / jnp.sum(s, axis=1, keepdims=True) for s in lane_sum]
        p_last = [p * r for p, r in zip(probs(last), inv_sum)]
        for h in range(_HEADS):
            i = h % _SUBLANES
            p_buf[h] = jnp.broadcast_to(p_last[h // _SUBLANES][i:i + 1], (_TILE, _TILE)).T
        acc = lax.fori_loop(
            num_chunks - _AHEAD_HIGH, last, lambda t, a: value_step(t, (a, zeros), ())[0], acc)
        out = [a * r for a, r in zip(acc, inv_sum)]

        def weighted(h, half, unit):
            return p_buf[h, pl.ds(half * _UNIT, _UNIT)] * unit.astype(jnp.float32)

        def add_head(h, rows):
            g = h // _SUBLANES
            total = out[g] + jnp.sum(rows, axis=0, keepdims=True)
            out[g] = jnp.where(sublane == h % _SUBLANES, total, out[g])

        wait(early_buf, early_sem)
        for b in range(_STRIDE):
            for seg in range(segs):
                h = seg * _STRIDE + b
                rows = weighted(h, 0, early_buf[b, seg])
                if seg >= _LOW_SEGS:
                    rows = rows + weighted(h, 1, early_buf[b, seg + segs - _LOW_SEGS])
                add_head(h, rows)
        for b in range(_STRIDE):
            wait(late_buf.at[b], late_sems.at[b])
            for seg in range(_LOW_SEGS):
                h = seg * _STRIDE + b
                add_head(h, weighted(h, 1, late_buf[b, seg]))
        o_buf[pl.ds(x * _HEADS, _HEADS)] = jnp.concatenate(out, axis=0).astype(o_buf.dtype)

    o_copy = pltpu.make_async_copy(o_buf, o_hbm, io_sem)
    o_copy.start()
    o_copy.wait()


@jax.jit
def pallas_standalone__mha_softmax__decode_kernel(q: jax.Array, k: jax.Array, v: jax.Array):
    batch, heads, q_len, dim = q.shape
    seq = k.shape[2]
    num_heads = batch * heads
    num_chunks = seq // _TILE
    assert q_len == 1 and dim == _TILE and num_heads % _HEADS == 0
    assert seq % _TILE == 0 and num_chunks > _NBUF and num_chunks & (num_chunks - 1) == 0
    segs = _HEADS // _STRIDE
    kv_shape = (num_heads // _STRIDE, _STRIDE * seq, dim)
    out = pl.pallas_call(
        _attention_kernel,
        in_specs=[pl.BlockSpec(memory_space=pl.ANY)] * 3,
        out_specs=pl.BlockSpec(memory_space=pl.ANY),
        out_shape=jax.ShapeDtypeStruct((num_heads, dim), q.dtype),
        scratch_shapes=[
            pltpu.VMEM((_NBUF, segs, _STRIDE, _TILE, dim), k.dtype),
            pltpu.VMEM((_STRIDE, 2 * segs - _LOW_SEGS, _UNIT, dim), v.dtype),
            pltpu.VMEM((_STRIDE, _LOW_SEGS, _UNIT, dim), v.dtype),
            pltpu.VMEM((num_heads, dim), q.dtype),
            pltpu.VMEM((num_chunks, _HEADS // _SUBLANES, _SUBLANES, _TILE), jnp.float32),
            pltpu.VMEM((_HEADS, _TILE, _TILE), jnp.float32),
            pltpu.VMEM((num_heads, dim), q.dtype),
            pltpu.SemaphoreType.DMA((_NBUF,)),
            pltpu.SemaphoreType.DMA(()),
            pltpu.SemaphoreType.DMA((_STRIDE,)),
            pltpu.SemaphoreType.DMA(()),
        ],
        compiler_params=pltpu.CompilerParams(
            disable_bounds_checks=True, disable_semaphore_checks=True),
    )(q.reshape(num_heads, dim), k.reshape(kv_shape), v.reshape(kv_shape))
    return out.reshape(q.shape)
```

```python
import math

import jax
import jax.numpy as jnp
from jax import lax
import jax.experimental.pallas as pl
import jax.experimental.pallas.tpu as pltpu

_HEADS = 8
_LANES = 2 * _HEADS
_UNIT = 64
_TILE = 2 * _UNIT
_PERIOD = 4
_LAG = 26
_AHEAD = 15
_NBUF = 16
_LATE = 7
_PIECE = 32

_QK_DIMS = (((1,), (1,)), ((), ()))
_PV_DIMS = (((1,), (0,)), ((), ()))


def _round_schedule():
    pairs = _LANES // _PERIOD
    schedule = []
    for i in range(pairs):
        rounds, pair = divmod(i - _LAG, pairs)
        schedule.append((pair * _PERIOD, 1, 0, _AHEAD + rounds))
        schedule.append((i * _PERIOD + 1, _PERIOD - 1, 1, _AHEAD))
    return schedule


def _fold(values, count):
    while len(values) > count:
        half = len(values) // 2
        values = [a + b for a, b in zip(values[:half], values[half:])]
    return values


def _attention_kernel(
    q_hbm, k_hbm, v_hbm, o_hbm,
    buf, late_buf, q_buf, s_buf, p_buf, o_buf,
    sems, late_sems, io_sem,
):
    num_heads, dim = q_hbm.shape
    num_passes = num_heads // _HEADS
    num_rounds = k_hbm.shape[1] // _UNIT
    exp2_scale = dim**-0.5 * math.log2(math.e)
    schedule = _round_schedule()
    aheads = sorted({ahead for *_, ahead in schedule}, reverse=True)

    def start(src, x, r, first, lanes, priority):
        slot = r & (_NBUF - 1)
        row = r * _UNIT if isinstance(r, int) else pl.multiple_of(r * _UNIT, _UNIT)
        pltpu.make_async_copy(
            src.at[pl.ds(x * _LANES + first, lanes), pl.ds(row, _UNIT)],
            buf.at[slot, pl.ds(first, lanes)],
            sems.at[slot],
        ).start(priority=priority)

    def wait(ref, sem):
        pltpu.make_async_copy(ref, ref, sem).wait()

    def advance(r, this, following=None, moved_on=()):
        slot = r & (_NBUF - 1)
        wait(buf.at[slot], sems.at[slot])
        for first, lanes, priority, ahead in schedule:
            if ahead in moved_on:
                start(*following, r + ahead - num_rounds, first, lanes, priority)
            else:
                start(*this, r + ahead, first, lanes, priority)

    def run_stream(step, carry, this, following):
        bounds = [0] + [num_rounds - ahead for ahead in aheads] + [num_rounds]
        for i in range(len(bounds) - 1):
            def body(r, c, moved_on=aheads[:i]):
                return step(r, c, lambda: advance(r, this, following, moved_on))
            carry = lax.fori_loop(bounds[i], bounds[i + 1], body, carry)
        return carry

    for r in range(-_AHEAD, 0):
        for first, lanes, priority, ahead in schedule:
            if r + ahead >= 0:
                start(k_hbm, 0, r + ahead, first, lanes, priority)
    q_copy = pltpu.make_async_copy(q_hbm, q_buf, io_sem)
    q_copy.start()
    q_copy.wait()

    q_f32 = q_buf[...].astype(jnp.float32)
    sublane = lax.broadcasted_iota(jnp.int32, (_HEADS, _TILE), 0)
    zeros = jnp.zeros((_HEADS, _TILE), jnp.float32)

    def per_head_matmul(lhs, r, dims, heads=_HEADS):
        out = None if heads == _HEADS else zeros
        for h in range(heads):
            tile = buf[r & (_NBUF - 1), pl.ds(2 * h, 2)].reshape(_TILE, dim)
            product = lax.dot_general(lhs, tile, dims, preferred_element_type=jnp.float32)
            out = product if out is None else jnp.where(sublane == h, product, out)
        return out

    outputs = []
    for x in range(num_passes):
        q = q_f32[x * _HEADS:(x + 1) * _HEADS].astype(q_buf.dtype)

        def score_step(r, lane_max, fetch):
            fetch()
            s = per_head_matmul(q, r, _QK_DIMS)
            s_buf[r] = s
            return jnp.maximum(lane_max, s)

        lane_max = run_stream(
            score_step, jnp.full((_HEADS, _TILE), -jnp.inf, jnp.float32), (k_hbm, x), (v_hbm, x))
        row_max = jnp.broadcast_to(jnp.max(lane_max, axis=1, keepdims=True), (_HEADS, _TILE))

        def probs(r):
            return jnp.exp2((s_buf[r] - row_max) * exp2_scale)

        def value_step(r, carry, fetch, heads=_HEADS):
            acc, lane_sum = carry
            p = probs(r)
            fetch()
            return acc + per_head_matmul(p.astype(buf.dtype), r, _PV_DIMS, heads), lane_sum + p

        if x + 1 < num_passes:
            acc, lane_sum = run_stream(value_step, (zeros, zeros), (v_hbm, x), (k_hbm, x + 1))
            outputs.append(acc / jnp.sum(lane_sum, axis=1, keepdims=True))

    x = num_passes - 1
    first_late = num_rounds - _LATE
    early_lanes = _LANES - 2
    late_units = [(half, r) for half in range(2) for r in range(first_late, num_rounds)]
    pieces = [(i, offset) for i in range(len(late_units)) for offset in range(0, _UNIT, _PIECE)]

    def heads_in(r):
        return _HEADS if r < first_late else _HEADS - 1

    def wait_round(r):
        slot = r & (_NBUF - 1)
        wait(buf.at[slot, pl.ds(0, 2 * heads_in(r))], sems.at[slot])

    def advance_to_end(r):
        wait_round(r)
        for first, lanes, priority, ahead in schedule:
            if r + ahead < first_late:
                start(v_hbm, x, r + ahead, first, lanes, priority)
            elif r + ahead < num_rounds:
                start(v_hbm, x, r + ahead, first, min(lanes, early_lanes - first), priority)
            elif priority == 1:
                i, offset = pieces.pop(0)
                half, late_round = late_units[i]
                pltpu.make_async_copy(
                    v_hbm.at[x * _LANES + early_lanes + half, pl.ds(late_round * _UNIT + offset, _PIECE)],
                    late_buf.at[i // 2, i % 2, pl.ds(offset, _PIECE)],
                    late_sems.at[i // 2],
                ).start(priority=1)

    carry = lax.fori_loop(
        0, first_late - _AHEAD,
        lambda r, c: value_step(r, c, lambda: advance(r, (v_hbm, x))),
        (zeros, zeros))
    issued = num_rounds - aheads[-1]
    for r in range(first_late - _AHEAD, issued):
        carry = value_step(r, carry, lambda: advance_to_end(r), heads_in(r))
    assert not pieces

    acc, lane_sum = carry
    for r in range(issued, num_rounds):
        lane_sum = lane_sum + probs(r)
    inv_sum = 1.0 / jnp.sum(lane_sum, axis=1, keepdims=True)
    for r in range(first_late, num_rounds):
        p = (probs(r) * inv_sum)[_HEADS - 1:]
        p_buf[r - first_late] = jnp.broadcast_to(p, (_TILE, _TILE)).T
    o_buf[pl.ds(0, num_heads - 2 * _HEADS)] = jnp.concatenate(outputs[:-1], axis=0).astype(o_buf.dtype)
    for r in range(issued, num_rounds):
        acc, _ = value_step(r, (acc, zeros), lambda: wait_round(r), heads_in(r))
    out = acc * inv_sum

    last_head = sublane == _HEADS - 1
    partial = [jnp.where(last_head, out, 0.0), zeros, zeros, zeros]
    for g in range(_LATE):
        wait(late_buf.at[g], late_sems.at[g])
        rows = []
        for j in range(2):
            half, r = late_units[2 * g + j]
            weighted = (
                p_buf[r - first_late, pl.ds(half * _UNIT, _UNIT)] * late_buf[g, j].astype(jnp.float32))
            rows += [weighted[i:i + _HEADS] for i in range(0, _UNIT, _HEADS)]
        partial = [a + b for a, b in zip(partial, _fold(rows, len(partial)))]
    out = jnp.where(last_head, jnp.sum(_fold(partial, 1)[0], axis=0, keepdims=True), out)

    o_buf[pl.ds(num_heads - 2 * _HEADS, 2 * _HEADS)] = (
        jnp.concatenate([outputs[-1], out], axis=0).astype(o_buf.dtype))
    o_copy = pltpu.make_async_copy(o_buf, o_hbm, io_sem)
    o_copy.start()
    o_copy.wait()


@jax.jit
def pallas_standalone__mha_softmax__decode_kernel(q: jax.Array, k: jax.Array, v: jax.Array):
    batch, heads, q_len, dim = q.shape
    seq = k.shape[2]
    num_heads = batch * heads
    num_rounds = seq // _TILE
    assert q_len == 1 and dim == _TILE and num_heads % (2 * _HEADS) == 0 and num_heads > 2 * _HEADS
    assert seq % (_TILE * _NBUF) == 0 and num_rounds > _AHEAD + _LATE
    kv_shape = (2 * num_heads, seq // 2, dim)
    out = pl.pallas_call(
        _attention_kernel,
        in_specs=[pl.BlockSpec(memory_space=pl.ANY)] * 3,
        out_specs=pl.BlockSpec(memory_space=pl.ANY),
        out_shape=jax.ShapeDtypeStruct((num_heads, dim), q.dtype),
        scratch_shapes=[
            pltpu.VMEM((_NBUF, _LANES, _UNIT, dim), k.dtype),
            pltpu.VMEM((_LATE, 2, _UNIT, dim), v.dtype),
            pltpu.VMEM((num_heads, dim), q.dtype),
            pltpu.VMEM((num_rounds, _HEADS, _TILE), jnp.float32),
            pltpu.VMEM((_LATE, _TILE, _TILE), jnp.float32),
            pltpu.VMEM((num_heads, dim), q.dtype),
            pltpu.SemaphoreType.DMA((_NBUF,)),
            pltpu.SemaphoreType.DMA((_LATE,)),
            pltpu.SemaphoreType.DMA(()),
        ],
        compiler_params=pltpu.CompilerParams(
            disable_bounds_checks=True, disable_semaphore_checks=True),
    )(q.reshape(num_heads, dim), k.reshape(kv_shape), v.reshape(kv_shape))
    return out.reshape(q.shape)
```

```python
import math

import jax
import jax.numpy as jnp
from jax import lax
import jax.experimental.pallas as pl
import jax.experimental.pallas.tpu as pltpu

_HEADS = 8
_RANGES = 2 * _HEADS
_UNIT = 64
_TILE = 2 * _UNIT
_PERIOD = 4
_LAG = 26
_AHEAD = 15
_NBUF = 16
_LATE = 7
_PIECE = 32

_QK_DIMS = (((1,), (1,)), ((), ()))
_PV_DIMS = (((1,), (0,)), ((), ()))


def _round_schedule():
    pairs = _RANGES // _PERIOD
    schedule = []
    for i in range(pairs):
        rounds, pair = divmod(i - _LAG, pairs)
        schedule.append((pair * _PERIOD, 1, 0, _AHEAD + rounds))
        schedule.append((i * _PERIOD + 1, _PERIOD - 1, 1, _AHEAD))
    return schedule


def _fold(values, count):
    while len(values) > count:
        half = len(values) // 2
        values = [a + b for a, b in zip(values[:half], values[half:])]
    return values


def _attention_kernel(
    q_hbm, k_hbm, v_hbm, o_hbm,
    buf, late_buf, q_buf, s_buf, p_buf, o_buf,
    sems, late_sems, io_sem,
):
    num_heads, dim = q_hbm.shape
    num_passes = num_heads // _HEADS
    num_rounds = k_hbm.shape[1] // _UNIT
    exp2_scale = dim**-0.5 * math.log2(math.e)
    schedule = _round_schedule()
    aheads = sorted({ahead for *_, ahead in schedule}, reverse=True)

    def start(src, x, r, first, count, priority):
        slot = r & (_NBUF - 1)
        row = r * _UNIT if isinstance(r, int) else pl.multiple_of(r * _UNIT, _UNIT)
        pltpu.make_async_copy(
            src.at[pl.ds(x * _RANGES + first, count), pl.ds(row, _UNIT)],
            buf.at[slot, pl.ds(first, count)],
            sems.at[slot],
        ).start(priority=priority)

    def wait(ref, sem):
        pltpu.make_async_copy(ref, ref, sem).wait()

    def advance(r, this, following=None, moved_on=()):
        slot = r & (_NBUF - 1)
        wait(buf.at[slot], sems.at[slot])
        for first, count, priority, ahead in schedule:
            if ahead in moved_on:
                start(*following, r + ahead - num_rounds, first, count, priority)
            else:
                start(*this, r + ahead, first, count, priority)

    def run_stream(step, carry, this, following):
        bounds = [0] + [num_rounds - ahead for ahead in aheads] + [num_rounds]
        for i in range(len(bounds) - 1):
            def body(r, c, moved_on=aheads[:i]):
                return step(r, c, lambda: advance(r, this, following, moved_on))
            carry = lax.fori_loop(bounds[i], bounds[i + 1], body, carry)
        return carry

    for r in range(-_AHEAD, 0):
        for first, count, priority, ahead in schedule:
            if r + ahead >= 0:
                start(k_hbm, 0, r + ahead, first, count, priority)
    q_copy = pltpu.make_async_copy(q_hbm, q_buf, io_sem)
    q_copy.start()
    q_copy.wait()

    q_f32 = q_buf[...].astype(jnp.float32)
    sublane = lax.broadcasted_iota(jnp.int32, (_HEADS, _TILE), 0)
    zeros = jnp.zeros((_HEADS, _TILE), jnp.float32)

    def per_head_matmul(lhs, r, dims, heads=_HEADS):
        out = None if heads == _HEADS else zeros
        for h in range(heads):
            tile = buf[r & (_NBUF - 1), pl.ds(2 * h, 2)].reshape(_TILE, dim)
            product = lax.dot_general(lhs, tile, dims, preferred_element_type=jnp.float32)
            out = product if out is None else jnp.where(sublane == h, product, out)
        return out

    outputs = []
    for x in range(num_passes):
        q = q_f32[x * _HEADS:(x + 1) * _HEADS].astype(q_buf.dtype)

        def score_step(r, lane_max, fetch):
            fetch()
            s = per_head_matmul(q, r, _QK_DIMS)
            s_buf[r] = s
            return jnp.maximum(lane_max, s)

        lane_max = run_stream(
            score_step, jnp.full((_HEADS, _TILE), -jnp.inf, jnp.float32), (k_hbm, x), (v_hbm, x))
        row_max = jnp.broadcast_to(jnp.max(lane_max, axis=1, keepdims=True), (_HEADS, _TILE))

        def probs(r):
            return jnp.exp2((s_buf[r] - row_max) * exp2_scale)

        def value_step(r, carry, fetch, heads=_HEADS):
            acc, lane_sum = carry
            p = probs(r)
            fetch()
            return acc + per_head_matmul(p.astype(buf.dtype), r, _PV_DIMS, heads), lane_sum + p

        if x + 1 < num_passes:
            acc, lane_sum = run_stream(value_step, (zeros, zeros), (v_hbm, x), (k_hbm, x + 1))
            outputs.append(acc / jnp.sum(lane_sum, axis=1, keepdims=True))

    x = num_passes - 1
    first_late = num_rounds - _LATE
    early_ranges = _RANGES - 2
    late_units = [(half, r) for half in range(2) for r in range(first_late, num_rounds)]
    pieces = [(i, offset) for i in range(len(late_units)) for offset in range(0, _UNIT, _PIECE)]

    def heads_in(r):
        return _HEADS if r < first_late else _HEADS - 1

    def wait_round(r):
        slot = r & (_NBUF - 1)
        wait(buf.at[slot, pl.ds(0, 2 * heads_in(r))], sems.at[slot])

    def advance_to_end(r):
        wait_round(r)
        for first, count, priority, ahead in schedule:
            if r + ahead < first_late:
                start(v_hbm, x, r + ahead, first, count, priority)
            elif r + ahead < num_rounds:
                start(v_hbm, x, r + ahead, first, min(count, early_ranges - first), priority)
            elif priority == 1:
                i, offset = pieces.pop(0)
                half, late_round = late_units[i]
                pltpu.make_async_copy(
                    v_hbm.at[x * _RANGES + early_ranges + half, pl.ds(late_round * _UNIT + offset, _PIECE)],
                    late_buf.at[i // 2, i % 2, pl.ds(offset, _PIECE)],
                    late_sems.at[i // 2],
                ).start(priority=1)

    carry = lax.fori_loop(
        0, first_late - _AHEAD,
        lambda r, c: value_step(r, c, lambda: advance(r, (v_hbm, x))),
        (zeros, zeros))
    issued = num_rounds - aheads[-1]
    for r in range(first_late - _AHEAD, issued):
        carry = value_step(r, carry, lambda: advance_to_end(r), heads_in(r))
    assert not pieces

    acc, lane_sum = carry
    for r in range(issued, num_rounds):
        lane_sum = lane_sum + probs(r)
    inv_sum = 1.0 / jnp.sum(lane_sum, axis=1, keepdims=True)
    for r in range(first_late, num_rounds):
        p = (probs(r) * inv_sum)[_HEADS - 1:]
        p_buf[r - first_late] = jnp.broadcast_to(p, (_TILE, _TILE)).T
    done, rest = pl.ds(0, num_heads - 2 * _HEADS), pl.ds(num_heads - 2 * _HEADS, 2 * _HEADS)
    o_buf[done] = jnp.concatenate(outputs[:-1], axis=0).astype(o_buf.dtype)
    for r in range(issued, num_rounds):
        acc, _ = value_step(r, (acc, zeros), lambda: wait_round(r), heads_in(r))
    out = acc * inv_sum
    pltpu.make_async_copy(o_buf.at[done], o_hbm.at[done], io_sem).start()

    last_head = sublane == _HEADS - 1
    partial = [jnp.where(last_head, out, 0.0), zeros, zeros, zeros]
    for g in range(_LATE):
        wait(late_buf.at[g], late_sems.at[g])
        rows = []
        for j in range(2):
            half, r = late_units[2 * g + j]
            weighted = (
                p_buf[r - first_late, pl.ds(half * _UNIT, _UNIT)] * late_buf[g, j].astype(jnp.float32))
            rows += [weighted[i:i + _HEADS] for i in range(0, _UNIT, _HEADS)]
        partial = [a + b for a, b in zip(partial, _fold(rows, len(partial)))]
    out = jnp.where(last_head, jnp.sum(_fold(partial, 1)[0], axis=0, keepdims=True), out)

    o_buf[rest] = jnp.concatenate([outputs[-1], out], axis=0).astype(o_buf.dtype)
    pltpu.make_async_copy(o_buf.at[rest], o_hbm.at[rest], io_sem).start()
    pltpu.make_async_copy(o_buf, o_hbm, io_sem).wait()


@jax.jit
def pallas_standalone__mha_softmax__decode_kernel(q: jax.Array, k: jax.Array, v: jax.Array):
    batch, heads, q_len, dim = q.shape
    seq = k.shape[2]
    num_heads = batch * heads
    num_rounds = seq // _TILE
    assert q_len == 1 and dim == _TILE and num_heads % (2 * _HEADS) == 0 and num_heads > 2 * _HEADS
    assert seq % (_TILE * _NBUF) == 0 and num_rounds > _AHEAD + _LATE
    kv_shape = (2 * num_heads, seq // 2, dim)
    out = pl.pallas_call(
        _attention_kernel,
        in_specs=[pl.BlockSpec(memory_space=pl.ANY)] * 3,
        out_specs=pl.BlockSpec(memory_space=pl.ANY),
        out_shape=jax.ShapeDtypeStruct((num_heads, dim), q.dtype),
        scratch_shapes=[
            pltpu.VMEM((_NBUF, _RANGES, _UNIT, dim), k.dtype),
            pltpu.VMEM((_LATE, 2, _UNIT, dim), v.dtype),
            pltpu.VMEM((num_heads, dim), q.dtype),
            pltpu.VMEM((num_rounds, _HEADS, _TILE), jnp.float32),
            pltpu.VMEM((_LATE, _TILE, _TILE), jnp.float32),
            pltpu.VMEM((num_heads, dim), q.dtype),
            pltpu.SemaphoreType.DMA((_NBUF,)),
            pltpu.SemaphoreType.DMA((_LATE,)),
            pltpu.SemaphoreType.DMA(()),
        ],
        compiler_params=pltpu.CompilerParams(
            disable_bounds_checks=True, disable_semaphore_checks=True),
    )(q.reshape(num_heads, dim), k.reshape(kv_shape), v.reshape(kv_shape))
    return out.reshape(q.shape)
```
